```python
import os as _os
_os.environ.setdefault('JAX_PLATFORMS', 'cpu')
import jax
import jax.numpy as jnp

def _softmax(x, axis=-1):
    return jax.nn.softmax(x, axis=axis)

def _gelu(x):
    return jax.nn.gelu(x, approximate=True)

def _silu(x):
    return jax.nn.silu(x)

def _sigmoid(x):
    return jax.nn.sigmoid(x)

def _layernorm(x, axis=-1, eps=1e-05):
    m = jnp.mean(x, axis=axis, keepdims=True)
    v = jnp.var(x, axis=axis, keepdims=True)
    return (x - m) / jnp.sqrt(v + eps)

def _scatter_add(tgt, idx, src, axis=0):
    return tgt.at[idx].add(src)

def _segment_sum(src, seg, n):
    return jax.ops.segment_sum(src, seg, n)

class _Rng:

    def __init__(self, key):
        self._k = key

    def _next(self):
        self._k, sub = jax.random.split(self._k)
        return sub

    def normal(self, shape):
        return jax.random.normal(self._next(), shape, dtype=jnp.bfloat16)

    def randint(self, lo, hi, shape):
        return jax.random.randint(self._next(), shape, lo, hi, dtype=jnp.int32)

    def uniform(self, shape, lo=0.0, hi=1.0):
        return jax.random.uniform(self._next(), shape, jnp.bfloat16, lo, hi)

    def permutation(self, n):
        return jax.random.permutation(self._next(), n)
kernel_name = 'concat_heads__ssm_conv_s5__memory_aug_recurrent_mem_tr__prompt'

def setup_inputs():
    _rng = _Rng(jax.random.key(int.from_bytes(__import__("os").urandom(4), "little")))
    _w = lambda a: (lambda t: t.astype(jnp.bfloat16) if jnp.issubdtype(t.dtype, jnp.floating) else t)(jnp.asarray(a))

    def _A_setup():
        B, S, D = (1, 2048, 1024)
        P = D
        Lambda_re = -0.5 * jnp.exp((lambda *s: _rng.normal(s) * 0.8)(P))
        Lambda_im = (lambda *s: _rng.normal(s) * 0.8)(P) * 1.0
        B_re = (lambda *s: _rng.normal(s) * 0.8)(P, D) * D ** (-0.5)
        B_im = (lambda *s: _rng.normal(s) * 0.8)(P, D) * D ** (-0.5)
        C_re = (lambda *s: _rng.normal(s) * 0.8)(D, P) * P ** (-0.5)
        C_im = (lambda *s: _rng.normal(s) * 0.8)(D, P) * P ** (-0.5)
        log_dt = (lambda *s: _rng.normal(s) * 0.8)(P) * 0.3 - 2.0
        Dskip = (lambda *s: _rng.normal(s) * 0.8)(D)
        return {'x': _w((lambda *s: _rng.normal(s) * 0.05)(B, S, D)), 'Lambda_re': _w(Lambda_re), 'Lambda_im': _w(Lambda_im), 'B_re': _w(B_re), 'B_im': _w(B_im), 'C_re': _w(C_re), 'C_im': _w(C_im), 'log_dt': _w(log_dt), 'Dskip': _w(Dskip)}
    _A_in = _A_setup()

    def _B_setup():
        B, S, Dm = (1, 2048, 1024)
        H, Dh = (32, 128)
        M, seg = (8, 32)
        seg = min(seg, S)
        S = S // seg * seg
        return {'x': _w((lambda *s: _rng.normal(s) * 0.05)(B, S, Dm)), 'mem0': _w((lambda *s: _rng.normal(s) * 0.8)(B, M, Dm)), 'Wq': _w((lambda *s: _rng.normal(s) * 1.6)(Dm, H, Dh) * Dm ** (-0.5)), 'Wk': _w((lambda *s: _rng.normal(s) * 1.6)(Dm, H, Dh) * Dm ** (-0.5)), 'Wv': _w((lambda *s: _rng.normal(s) * 0.8)(Dm, H, Dh) * Dm ** (-0.5)), 'Wo': _w((lambda *s: _rng.normal(s) * 0.8)(H, Dh, Dm) * (H * Dh) ** (-0.5)), 'seg_len': seg}
    _B_in = _B_setup()
    return {'A_x': _A_in['x'], 'A_Lambda_re': _A_in['Lambda_re'], 'A_Lambda_im': _A_in['Lambda_im'], 'A_B_re': _A_in['B_re'], 'A_B_im': _A_in['B_im'], 'A_C_re': _A_in['C_re'], 'A_C_im': _A_in['C_im'], 'A_log_dt': _A_in['log_dt'], 'A_Dskip': _A_in['Dskip'], 'B_x': _B_in['x'], 'B_mem0': _B_in['mem0'], 'B_Wq': _B_in['Wq'], 'B_Wk': _B_in['Wk'], 'B_Wv': _B_in['Wv'], 'B_Wo': _B_in['Wo'], 'B_seg_len': _B_in['seg_len']}

def reference(A_x, A_Lambda_re, A_Lambda_im, A_B_re, A_B_im, A_C_re, A_C_im, A_log_dt, A_Dskip, B_x, B_mem0, B_Wq, B_Wk, B_Wv, B_Wo, B_seg_len):

    def _A_ref(x, Lambda_re, Lambda_im, B_re, B_im, C_re, C_im, log_dt, Dskip):
        Bsz, L, H = x.shape
        Lam = Lambda_re + 1j * Lambda_im
        Bmat = B_re + 1j * B_im
        Cmat = C_re + 1j * C_im
        dt = jnp.exp(log_dt)
        Lam_bar = jnp.exp(dt * Lam)
        B_bar = ((Lam_bar - 1.0) / Lam)[:, None] * Bmat
        Bu = jnp.einsum('bld,pd->blp', x + 0j, B_bar)
        h = jnp.zeros_like(Bu[:, 0, :])
        hs = []
        for t in range(L):
            h = Lam_bar[None, :] * h + Bu[:, t, :]
            hs.append(h)
        hseq = jnp.stack(hs, 1)
        y = 2.0 * jnp.einsum('blp,dp->bld', hseq, Cmat).real + x * Dskip[None, None, :]
        return y

    def _B_ref(x, mem0, Wq, Wk, Wv, Wo, seg_len):
        B, S, Dm = x.shape
        H, Dh = (Wq.shape[1], Wq.shape[2])
        M = mem0.shape[1]
        scale = Dh ** (-0.5)
        n_seg = S // seg_len
        L = M + seg_len
        idx = jnp.arange(L)
        mask = (idx[:, None] < M) | (idx[:, None] >= idx[None, :])
        mem = mem0
        outs = []
        for s in range(n_seg):
            xs = x[:, s * seg_len:(s + 1) * seg_len, :].copy()
            h = jnp.concatenate([mem, xs], axis=1)
            q = jnp.einsum('btd,dhe->bhte', h, Wq)
            k = jnp.einsum('btd,dhe->bhte', h, Wk)
            v = jnp.einsum('btd,dhe->bhte', h, Wv)
            scores = jnp.einsum('bhqe,bhke->bhqk', q, k) * scale
            scores = jnp.where(mask[None, None], scores, -1000000000.0)
            p = _softmax(scores, axis=-1)
            o = jnp.einsum('bhqk,bhke->bhqe', p, v)
            o = jnp.einsum('bhte,hed->btd', o, Wo)
            mem = o[:, :M, :].copy()
            outs.append(o[:, M:, :])
        return jnp.concatenate(outs, axis=1)
    a = _A_ref(A_x, A_Lambda_re, A_Lambda_im, A_B_re, A_B_im, A_C_re, A_C_im, A_log_dt, A_Dskip)
    b = _B_ref(B_x, B_mem0, B_Wq, B_Wk, B_Wv, B_Wo, B_seg_len)
    return jnp.concatenate([a, b], axis=-1)
```

```python
import functools
import math

import jax
import jax.numpy as jnp
import jax.experimental.pallas as pl
import jax.experimental.pallas.tpu as pltpu

F32 = jnp.float32
BF16 = jnp.bfloat16
U32 = jnp.uint32

S = 2048
D = 1024
H = 32
DH = 128
M = 8
SEG = 32
L = M + SEG
NB = D // 128
PAIR = 2 * SEG
N_PAIR = S // PAIR

SLAB = 520
TA = 128
TAP = TA + 8
N_CH = S // TA
NQ = 4
TY = S // NQ

NT = (((1,), (1,)), ((), ()))


def _kernel(xa_hbm, lre_ref, lim_ref, bre_hbm, bim_hbm, cre_hbm, cim_hbm, ldt_ref, dsk_ref,
            xb_hbm, mem0_ref, wq_hbm, wk_hbm, wv_hbm, wo_hbm,
            out_hbm,
            xa_s, xb_s, bc_s, wraw_s, woraw_s, w_s, wo_s, h_s, ya_s, ob_s,
            sr0, si0, sr1, si1, sv_s, o_s, df_s, acc_s,
            in_sem, w_sem, out_sem):
    XA0 = 2 * TA
    cp_xa0 = pltpu.make_async_copy(xa_hbm.at[pl.ds(0, XA0), :], xa_s.at[pl.ds(0, XA0), :], in_sem.at[0])
    cp_xa1 = pltpu.make_async_copy(xa_hbm.at[pl.ds(XA0, S - XA0), :], xa_s.at[pl.ds(XA0, S - XA0), :],
                                   in_sem.at[6])
    cp_bc = [pltpu.make_async_copy(src, bc_s.at[i], in_sem.at[1 + i])
             for i, src in enumerate((bre_hbm, bim_hbm, cre_hbm, cim_hbm))]
    cp_xb = pltpu.make_async_copy(xb_hbm, xb_s, in_sem.at[5])
    wrows = D * H // NQ
    worows = H * DH // NQ

    def cp_w(m, c):
        if m == 3:
            return pltpu.make_async_copy(wo_hbm.at[pl.ds(c * worows, worows), :],
                                         woraw_s.at[pl.ds(c * worows, worows), :],
                                         w_sem.at[c * 4 + m])
        src = (wq_hbm, wk_hbm, wv_hbm)[m]
        return pltpu.make_async_copy(src.at[pl.ds(c * wrows, wrows), :],
                                     wraw_s.at[m, pl.ds(c * wrows, wrows), :],
                                     w_sem.at[c * 4 + m])

    cp_xa0.start()
    cp_bc[0].start()
    cp_bc[1].start()

    lre = lre_ref[...].astype(F32)
    lim = lim_ref[...].astype(F32)
    dt = jnp.exp(ldt_ref[...].astype(F32)).astype(BF16).astype(F32)
    mag = jnp.exp(dt * lre)
    ang = dt * lim
    lb_re = mag * jnp.cos(ang)
    lb_im = mag * jnp.sin(ang)
    nr = lb_re - 1.0
    den = lre * lre + lim * lim
    cf_re = 2.0 * (nr * lre + lb_im * lim) / den
    cf_im = 2.0 * (lb_im * lre - nr * lim) / den
    dsk = dsk_ref[...].astype(F32)

    scan_bufs = ((sr0, si0), (sr1, si1))

    def bu_chunk(c, u):
        x = xa_s[pl.ds(pl.multiple_of(c * TA, TA), TA), :]
        for buf, widx in zip(scan_bufs[u], (0, 1)):
            for n in range(NB):
                buf[n * TAP:n * TAP + TA, :] = jax.lax.dot_general(
                    x, bc_s[widx, n * 128:(n + 1) * 128, :], NT, preferred_element_type=F32)

    def scan_chunk(c, u, gr, gi):
        sr, si = scan_bufs[u]
        for t in range(TA):
            ur = sr[pl.ds(t, NB, stride=TAP), :]
            ui = si[pl.ds(t, NB, stride=TAP), :]
            vr = cf_re * ur - cf_im * ui
            vi = cf_re * ui + cf_im * ur
            gr, gi = (lb_re * gr + lb_im * gi) + vr, (lb_re * gi - lb_im * gr) - vi
            sr[pl.ds(t, NB, stride=TAP), :] = gr
            si[pl.ds(t, NB, stride=TAP), :] = gi
        r0 = pl.multiple_of(c * (TA // 2), TA // 2)
        for k, buf in enumerate((sr, si)):
            for n in range(NB):
                h_s[k * NB + n, pl.ds(r0, TA // 2), :] = pltpu.bitcast(
                    buf[n * TAP:n * TAP + TA, :].astype(BF16), U32)
        return gr, gi

    cp_xa0.wait()
    cp_bc[0].wait()
    cp_bc[1].wait()
    cp_xa1.start()
    cp_bc[2].start()
    cp_bc[3].start()

    zero = jnp.zeros((NB, 128), F32)
    bu_chunk(0, 0)
    bu_chunk(1, 1)
    g0 = scan_chunk(0, 0, zero, zero)

    cp_xa1.wait()
    for c in range(NQ):
        for m in range(4):
            cp_w(m, c).start()
    cp_xb.start()

    def a1_body(i, carry):
        gr, gi = carry
        bu_chunk(2 * i, 0)
        gr, gi = scan_chunk(2 * i - 1, 1, gr, gi)
        bu_chunk(2 * i + 1, 1)
        gr, gi = scan_chunk(2 * i, 0, gr, gi)
        return gr, gi

    gr, gi = jax.lax.fori_loop(1, N_CH // 2, a1_body, g0)
    scan_chunk(N_CH - 1, 1, gr, gi)

    cp_bc[2].wait()
    cp_bc[3].wait()

    def a2_body(q, carry):
        for m in range(4):
            cp_w(m, q).wait()
        for u in range(TY // 256):
            base = pl.multiple_of(q * TY + u * 256, 256)
            hb = pl.multiple_of(q * (TY // 2) + u * 128, 128)
            hr = jnp.concatenate([pltpu.bitcast(h_s[n, pl.ds(hb, 128), :], BF16) for n in range(NB)], axis=1)
            hi = jnp.concatenate([pltpu.bitcast(h_s[NB + n, pl.ds(hb, 128), :], BF16) for n in range(NB)],
                                 axis=1)
            for n in range(NB):
                y = jax.lax.dot_general(hr, bc_s[2, n * 128:(n + 1) * 128, :], NT,
                                        preferred_element_type=F32)
                y = y + jax.lax.dot_general(hi, bc_s[3, n * 128:(n + 1) * 128, :], NT,
                                            preferred_element_type=F32)
                y = y + xa_s[pl.ds(base, 256), n * 128:(n + 1) * 128].astype(F32) * dsk[n:n + 1, :]
                ya_s[pl.ds(base, 256), n * 128:(n + 1) * 128] = y
        npair = D // 2 // NQ
        for m in range(3):
            for u in range(npair):
                dp = q * npair + u
                w = pltpu.bitcast(wraw_s[m, pl.ds(pl.multiple_of(dp * 64, 64), 64), :], U32)
                e = w[0:16]
                o = w[16:32]
                lo = (e & jnp.uint32(0xFFFF)) | (o << 16)
                hi = (e >> 16) | (o & jnp.uint32(0xFFFF0000))
                w_s[pl.ds(m * H * SLAB + dp, 16, stride=SLAB), :] = lo
                w_s[pl.ds((m * H + 16) * SLAB + dp, 16, stride=SLAB), :] = hi
        for u in range(worows // 128):
            r0 = pl.multiple_of(q * worows + u * 128, 128)
            r1 = pl.multiple_of(q * (worows // 2) + u * 64, 64)
            for n in range(NB):
                wo_s[n, pl.ds(r1, 64), :] = pltpu.bitcast(
                    woraw_s[pl.ds(r0, 128), n * 128:(n + 1) * 128], U32)
        base = pl.multiple_of(q * TY, TY)
        pltpu.make_async_copy(ya_s.at[pl.ds(base, TY), :],
                              out_hbm.at[pl.ds(base, TY), pl.ds(0, D)],
                              out_sem.at[0]).start()
        return carry

    jax.lax.fori_loop(0, NQ, a2_body, 0)
    cp_xb.wait()

    row = jax.lax.broadcasted_iota(jnp.int32, (L, L), 0)
    col = jax.lax.broadcasted_iota(jnp.int32, (L, L), 1)
    mask = (row < M) | (row >= col)
    exp_c = (DH ** -0.5) * math.log2(math.e)

    def proj(lhs, m, h):
        idx = m * H + (h % 2) * 16 + h // 2
        w = pltpu.bitcast(w_s[idx * SLAB:idx * SLAB + 512, :], BF16)
        return jnp.dot(lhs, w, preferred_element_type=F32)

    S_LAG = 1
    V_LAG = 4
    H_EARLY = 24

    def segment(lhs, first):
        qs, ks, vs, ps = {}, {}, {}, {}

        def stage_p(h):
            vals = []
            for m in range(3):
                r = proj(lhs, m, h)
                if first:
                    sv_s[m * H + h] = r[L:L + 8]
                    r = r[0:L]
                else:
                    r = jnp.concatenate([r[0:M], sv_s[m * H + h], r[M:]], axis=0)
                vals.append(r.astype(BF16))
            qs[h], ks[h], vs[h] = vals

        def stage_s(h):
            s = jax.lax.dot_general(qs.pop(h), ks.pop(h), NT, preferred_element_type=F32)
            s = jnp.where(mask, s, -1e9)
            mx = jnp.max(s, axis=-1, keepdims=True)
            p = jnp.exp2((s - mx) * exp_c)
            l = jnp.sum(p, axis=-1, keepdims=True)
            r = pl.reciprocal(l, approx=True)
            r = r * (2.0 - l * r)
            ps[h] = (p * r).astype(BF16)

        def stage_v(h):
            o = jnp.dot(ps.pop(h), vs.pop(h), preferred_element_type=F32)
            if first:
                df_s[h] = o[32:40]
                o_s[h, 0:16, :] = pltpu.bitcast(o[0:32].astype(BF16), U32)
            else:
                o_s[h] = pltpu.bitcast(jnp.concatenate([o, df_s[h]], axis=0).astype(BF16), U32)

        rows = 32 if first else 48

        def wo_part(n, h0, h1):
            o = jnp.concatenate([pltpu.bitcast(o_s[h, 0:rows // 2, :], BF16) for h in range(h0, h1)], axis=1)
            w = pltpu.bitcast(wo_s[n, h0 * DH // 2:h1 * DH // 2, :], BF16)
            return jnp.dot(o, w, preferred_element_type=F32)

        def wo_early(n):
            acc_s[0:rows, n * 128:(n + 1) * 128] = wo_part(n, 0, H_EARLY)

        for step in range(H + V_LAG):
            if step < H:
                stage_p(step)
            else:
                wo_early(step - H)
            if 0 <= step - S_LAG < H:
                stage_s(step - S_LAG)
            if 0 <= step - V_LAG < H:
                stage_v(step - V_LAG)
        for n in range(V_LAG, NB):
            wo_early(n)
        late = jnp.concatenate([wo_part(n, H_EARLY, H) for n in range(NB)], axis=1)
        return jnp.concatenate([late[0:M] + acc_s[0:M, :], late[M:rows] + acc_s[M:rows, :]], axis=0)

    def b_body(j, mem):
        base = pl.multiple_of(j * PAIR, PAIR)
        x = xb_s[pl.ds(base, PAIR), :].astype(F32)
        lhs = jnp.concatenate([mem, x[0:40]], axis=0).astype(BF16)
        res = segment(lhs, True)
        ob_s[pl.ds(base, 24), :] = res[8:32]
        lhs = jnp.concatenate([res[0:M], x[40:64]], axis=0).astype(BF16)
        res = segment(lhs, False)
        ob_s[pl.ds(base + 32, 32), :] = res[8:40]
        ob_s[pl.ds(base + 24, 8), :] = res[40:48]
        pltpu.make_async_copy(ob_s.at[pl.ds(base, PAIR), :],
                              out_hbm.at[pl.ds(base, PAIR), pl.ds(D, D)],
                              out_sem.at[1]).start()
        return res[0:M]

    jax.lax.fori_loop(0, N_PAIR, b_body, mem0_ref[...].astype(F32))

    pltpu.make_async_copy(ya_s, out_hbm.at[:, pl.ds(0, D)], out_sem.at[0]).wait()
    pltpu.make_async_copy(ob_s, out_hbm.at[:, pl.ds(D, D)], out_sem.at[1]).wait()


@functools.partial(jax.jit, static_argnames=("B_seg_len",))
def pallas_concat_heads__ssm_conv_s5__memory_aug_recurrent_mem_tr__prompt_kernel(
    A_x: jax.Array,
    A_Lambda_re: jax.Array,
    A_Lambda_im: jax.Array,
    A_B_re: jax.Array,
    A_B_im: jax.Array,
    A_C_re: jax.Array,
    A_C_im: jax.Array,
    A_log_dt: jax.Array,
    A_Dskip: jax.Array,
    B_x: jax.Array,
    B_mem0: jax.Array,
    B_Wq: jax.Array,
    B_Wk: jax.Array,
    B_Wv: jax.Array,
    B_Wo: jax.Array,
    B_seg_len: int,
):
    assert B_seg_len == SEG
    assert A_x.shape == (1, S, D) and B_x.shape == (1, S, D)
    assert B_Wq.shape == (D, H, DH) and B_Wo.shape == (H, DH, D) and B_mem0.shape == (1, M, D)

    hbm = pl.BlockSpec(memory_space=pl.ANY)
    vmem = pl.BlockSpec(memory_space=pltpu.VMEM)
    out = pl.pallas_call(
        _kernel,
        out_shape=jax.ShapeDtypeStruct((S, 2 * D), F32),
        in_specs=[hbm, vmem, vmem, hbm, hbm, hbm, hbm, vmem, vmem,
                  hbm, vmem, hbm, hbm, hbm, hbm],
        out_specs=hbm,
        scratch_shapes=[
            pltpu.VMEM((S, D), BF16),
            pltpu.VMEM((S, D), BF16),
            pltpu.VMEM((4, D, D), BF16),
            pltpu.VMEM((3, D * H, DH), BF16),
            pltpu.VMEM((H * DH, D), BF16),
            pltpu.VMEM((3 * H * SLAB, 128), U32),
            pltpu.VMEM((NB, H * DH // 2, 128), U32),
            pltpu.VMEM((2 * NB, S // 2, 128), U32),
            pltpu.VMEM((S, D), F32),
            pltpu.VMEM((S, D), F32),
            pltpu.VMEM((NB * TAP, 128), F32),
            pltpu.VMEM((NB * TAP, 128), F32),
            pltpu.VMEM((NB * TAP, 128), F32),
            pltpu.VMEM((NB * TAP, 128), F32),
            pltpu.VMEM((3 * H, 8, 128), F32),
            pltpu.VMEM((H, 24, 128), U32),
            pltpu.VMEM((H, 8, 128), F32),
            pltpu.VMEM((48, D), F32),
            pltpu.SemaphoreType.DMA((7,)),
            pltpu.SemaphoreType.DMA((4 * NQ,)),
            pltpu.SemaphoreType.DMA((2,)),
        ],
        compiler_params=pltpu.CompilerParams(vmem_limit_bytes=120 * 1024 * 1024),
    )(
        A_x.reshape(S, D),
        A_Lambda_re.reshape(NB, 128),
        A_Lambda_im.reshape(NB, 128),
        A_B_re, A_B_im, A_C_re, A_C_im,
        A_log_dt.reshape(NB, 128),
        A_Dskip.reshape(NB, 128),
        B_x.reshape(S, D),
        B_mem0.reshape(M, D),
        B_Wq.reshape(D * H, DH),
        B_Wk.reshape(D * H, DH),
        B_Wv.reshape(D * H, DH),
        B_Wo.reshape(H * DH, D),
    )
    return out.reshape(1, S, 2 * D)
```

```python
import math

import jax
import jax.numpy as jnp
import jax.experimental.pallas as pl
import jax.experimental.pallas.tpu as pltpu

F32 = jnp.float32
BF16 = jnp.bfloat16
U32 = jnp.uint32

S = 2048
D = 1024
H = 32
DH = 128
M = 8
SEG = 32
L = M + SEG
NB = D // 128
PAIR = 2 * SEG
N_PAIR = S // PAIR
B_UNROLL = 2

SLAB = 516
W0 = 8
TA = 128
TAP = TA + 8
N_CH = S // TA
NQ = 8
TY = S // NQ
HP = S // 2 + 8
WOP = H * DH // 2

NT = (((1,), (1,)), ((), ()))


def _kernel(xa_hbm, lre_hbm, lim_hbm, bre_hbm, bim_hbm, cre_hbm, cim_hbm, ldt_hbm, dsk_hbm,
            xb_hbm, mem0_hbm, wq_hbm, wk_hbm, wv_hbm, wo_hbm,
            out_hbm,
            xa_s, xb_s, bc_s, wraw_s, woraw_s, w_s, wo_s, h_s, ya_s, ob_s,
            sb0, sb1, sv_s, o_s, acc_s, pre_s, par_s, mem0_s, z_s,
            in_sem, out_sem):
    def cp_xa(i):
        r0 = pl.multiple_of(i * (2 * TA), 2 * TA)
        return pltpu.make_async_copy(xa_hbm.at[pl.ds(r0, 2 * TA), :], xa_s.at[pl.ds(r0, 2 * TA), :],
                                     in_sem.at[10 + i])

    def cp_b(g, src=None):
        r0 = g * 256
        if src is None:
            r0 = pl.multiple_of(r0, 256)
            src = bre_hbm.at[pl.ds(0, 256), :]
        return pltpu.make_async_copy(src, bc_s.at[pl.ds(r0, 256), :], in_sem.at[18 + g])

    cp_small = [pltpu.make_async_copy(src, dst, in_sem.at[2 + i]) for i, (src, dst) in enumerate(
        ((lre_hbm, par_s.at[0]), (lim_hbm, par_s.at[1]), (ldt_hbm, par_s.at[2]), (dsk_hbm, par_s.at[3]),
         (mem0_hbm, mem0_s)))]
    cp_c = [pltpu.make_async_copy(src, bc_s.at[pl.ds((2 + i) * D, D), :], in_sem.at[7 + i])
            for i, src in enumerate((cre_hbm, cim_hbm))]
    cp_xb = pltpu.make_async_copy(xb_hbm, xb_s, in_sem.at[9])
    wrows = D * H // NQ
    worows = H * DH // NQ

    def cp_w(m, c):
        if m == 3:
            return pltpu.make_async_copy(wo_hbm.at[pl.ds(c * worows, worows), :],
                                         woraw_s.at[pl.ds(c * worows, worows), :],
                                         in_sem.at[32 + c * 4 + m])
        src = (wq_hbm, wk_hbm, wv_hbm)[m]
        return pltpu.make_async_copy(src.at[pl.ds(c * wrows, wrows), :],
                                     wraw_s.at[m, pl.ds(c * wrows, wrows), :],
                                     in_sem.at[32 + c * 4 + m])

    cp_xa(0).start()
    for g in range(NB):
        cp_b(g, (bre_hbm, bim_hbm)[g // 4].at[pl.ds((g % 4) * 256, 256), :]).start()
        if g == 0:
            for c in cp_small:
                c.start()
    for i in range(1, N_CH // 2):
        cp_xa(i).start()
    for c in cp_c:
        c.start()
    for c in range(NQ):
        for m in range(4):
            cp_w(m, c).start()
    cp_xb.start()

    scan_bufs = (sb0, sb1)
    z_s[0] = 0
    zrow = {id(w_s): W0 + 3 * H * SLAB, id(wo_s): NB * WOP, id(h_s): 2 * NB * HP}
    for ref in (w_s, wo_s, h_s):
        ref[zrow[id(ref)]:zrow[id(ref)] + 8, :] = jnp.zeros((8, 128), ref.dtype)

    def token(*refs):
        tok = None
        for ref in refs:
            t = ref[pl.ds(pl.multiple_of(zoff + zrow[id(ref)], 8), 8), :]
            tok = t if tok is None else tok | t
        return tok

    def after(blocks, toks):
        blocks = list(blocks)
        for b, tok in toks.items():
            blocks[b] = jnp.concatenate([blocks[b][0:8] | tok, blocks[b][8:]], axis=0)
        return jnp.concatenate([pltpu.bitcast(b, BF16) for b in blocks], axis=1)

    def pack2(a, b):
        r = pltpu.bitcast(jnp.concatenate([a, b], axis=0).astype(BF16).astype(F32), U32)
        return (r[0:8] >> 16) | r[8:16]

    def scan_steps(c, u, t0, t1, gr, gi, toff=0):
        sb = scan_bufs[u]
        for t in range(t0, t1, 2):
            out = []
            for tt in (t, t + 1):
                ur = sb[pl.ds(toff + tt, NB, stride=TAP), :]
                ui = sb[pl.ds(toff + tt + NB * TAP, NB, stride=TAP), :]
                vr = cf_re * ur - cf_im * ui
                vi = cf_re * ui + cf_im * ur
                gr, gi = (lb_re * gr + lb_im * gi) + vr, (lb_re * gi - lb_im * gr) - vi
                out.append((gr, gi))
            row = c * (TA // 2) + (toff + t) // 2
            h_s[pl.ds(row, NB, stride=HP), :] = pack2(out[0][0], out[1][0])
            h_s[pl.ds(row + NB * HP, NB, stride=HP), :] = pack2(out[0][1], out[1][1])
        return gr, gi

    SCAN_END = [min(TA, 2 * -(-(k + 1) * TA // 2 // 14)) for k in range(2 * NB)]

    def bu_and_scan(cb, ub, cs, us, gr, gi):
        r0 = pl.multiple_of(cb * TA, TA)
        xblk = [pltpu.bitcast(xa_s[pl.ds(r0, TA), n * 128:(n + 1) * 128], U32) for n in range(NB)]
        zero_bits = token(h_s)
        toks = [{}, {}]
        done = 0
        for i in range(2 * NB):
            r = jax.lax.dot_general(after(xblk, toks.pop(0)), bc_s[i * 128:(i + 1) * 128, :], NT,
                                    preferred_element_type=F32)
            scan_bufs[ub][i * TAP:i * TAP + TA, :] = r
            toks.append({})
            if done < SCAN_END[i]:
                gr = gr + pltpu.bitcast(pltpu.bitcast(r[0:8], U32) & zero_bits, F32)
                gr, gi = scan_steps(cs, us, done, SCAN_END[i], gr, gi)
                done = SCAN_END[i]
                toks[1] = {4: token(h_s)}
        assert done == TA
        return gr, gi

    def bu_dot(c, b):
        w0, s0 = b * 128, b * TAP
        if not isinstance(b, int):
            w0, s0 = pl.multiple_of(w0, 128), pl.multiple_of(s0, 8)
        r = jax.lax.dot_general(xa_s[c * TA:(c + 1) * TA, :], bc_s[pl.ds(w0, 128), :], NT,
                                preferred_element_type=F32)
        scan_bufs[c][pl.ds(s0, TA), :] = r
        return r

    def pro_body(g, carry):
        cp_b(g).wait()
        for b in (2 * g, 2 * g + 1):
            for c in range(2):
                bu_dot(c, b)
        return carry

    cp_xa(0).wait()
    jax.lax.fori_loop(0, NB - 1, pro_body, 0)
    cp_b(NB - 1).wait()
    for c in cp_small:
        c.wait()
    zoff = z_s[0]
    lre = par_s[0].astype(F32)
    lim = par_s[1].astype(F32)
    dt = jnp.exp(par_s[2].astype(F32)).astype(BF16).astype(F32)
    mag = jnp.exp(dt * lre)
    ang = dt * lim
    lb_re = mag * jnp.cos(ang)
    lb_im = mag * jnp.sin(ang)
    nr = lb_re - 1.0
    den = lre * lre + lim * lim
    cf_re = 2.0 * (nr * lre + lb_im * lim) / den
    cf_im = 2.0 * (lb_im * lre - nr * lim) / den
    dsk = par_s[3].astype(F32)
    for c in range(2):
        for b in (2 * NB - 2, 2 * NB - 1):
            bu_dot(c, b)
    gr = gi = jnp.zeros((NB, 128), F32)
    gr, gi = scan_steps(0, 0, 0, TA, gr, gi)
    g0 = (gr, gi)

    def a1_body(i, carry):
        cp_xa(i).wait()
        gr, gi = carry
        gr, gi = bu_and_scan(2 * i, 0, 2 * i - 1, 1, gr, gi)
        gr, gi = bu_and_scan(2 * i + 1, 1, 2 * i, 0, gr, gi)
        return gr, gi

    g1 = jax.lax.fori_loop(1, N_CH // 2, a1_body, g0)
    for c in cp_c:
        c.wait()

    def a2_body(q, carry):
        for m in range(4):
            cp_w(m, q).wait()
        npair = D // 2 // NQ
        gr, gi = carry

        def rl_w(u):
            dp = q * npair + u
            rows = [dp]
            if u >= npair - 4:
                rows.append(jnp.where(q == NQ - 1, dp - D // 2, dp))
            for m in range(3):
                w = pltpu.bitcast(wraw_s[m, pl.ds(pl.multiple_of(dp * 64, 64), 64), :], U32)
                e = w[0:16]
                o = w[16:32]
                lo = (e & jnp.uint32(0xFFFF)) | (o << 16)
                hi = (e >> 16) | (o & jnp.uint32(0xFFFF0000))
                for r in rows:
                    w_s[pl.ds(W0 + m * H * SLAB + r, 16, stride=SLAB), :] = lo
                    w_s[pl.ds(W0 + (m * H + 16) * SLAB + r, 16, stride=SLAB), :] = hi

        def rl_wo(u):
            r0 = pl.multiple_of(q * worows + (u // 4) * 32, 32)
            r1 = pl.multiple_of(q * (worows // 2) + (u // 4) * 16, 16)
            for n in range(2 * (u % 4), 2 * (u % 4) + 2):
                wo_s[pl.ds(n * WOP + r1, 16), :] = pltpu.bitcast(
                    woraw_s[pl.ds(r0, 32), n * 128:(n + 1) * 128], U32)

        todo = list(range(npair))

        def piece():
            for _ in range(2 if len(todo) % (npair // 4) == 0 else 1):
                u = todo.pop(0)
                rl_w(u)
                rl_wo(u)
            return token(w_s, wo_s)

        toks_r, toks_i = {}, {}
        zero_bits = jnp.concatenate([token(h_s)] * (TA // 16), axis=0)
        for u in range(TY // TA):
            base = pl.multiple_of(q * TY + u * TA, TA)
            hb = pl.multiple_of(q * (TY // 2) + u * (TA // 2), TA // 2)
            hr = [h_s[pl.ds(n * HP + hb, TA // 2), :] for n in range(NB)]
            hi = [h_s[pl.ds((NB + n) * HP + hb, TA // 2), :] for n in range(NB)]
            hr = [v | zero_bits for v in hr]
            hi = [v | zero_bits for v in hi]
            for n in range(NB):
                y = jax.lax.dot_general(after(hr, toks_r), bc_s[2 * D + n * 128:2 * D + (n + 1) * 128, :], NT,
                                        preferred_element_type=F32)
                y = y + jax.lax.dot_general(after(hi, toks_i), bc_s[3 * D + n * 128:3 * D + (n + 1) * 128, :], NT,
                                            preferred_element_type=F32)
                y = y + xa_s[pl.ds(base, TA), n * 128:(n + 1) * 128].astype(F32) * dsk[n:n + 1, :]
                ya_s[pl.ds(base, TA), n * 128:(n + 1) * 128] = y
                if u == 0 and n < TA // NQ // 4:
                    gr = gr + pltpu.bitcast(pltpu.bitcast(y[0:8], U32) & zero_bits[0:8], F32)
                    gr, gi = scan_steps(N_CH - 1, 1, 4 * n, 4 * n + 4, gr, gi, q * (TA // NQ))
                if todo:
                    toks_i = {0: piece(), 4: piece()}
                    toks_r = {0: piece(), 4: piece()}
        assert not todo
        base = pl.multiple_of(q * TY, TY)
        pltpu.make_async_copy(ya_s.at[pl.ds(base, TY), :],
                              out_hbm.at[pl.ds(base, TY), pl.ds(0, D)],
                              out_sem.at[0]).start()
        return gr, gi

    jax.lax.fori_loop(0, NQ, a2_body, g1)
    cp_xb.wait()

    def iota2(shape):
        return (jax.lax.broadcasted_iota(jnp.int32, shape, 0),
                jax.lax.broadcasted_iota(jnp.int32, shape, 1))

    r, c = iota2((32, 48))
    mask_a = (c < L) & ((r < M) | (r >= c))
    r, c = iota2((48, 80))
    mem_b = (c >= 48) & (c < 56)
    mask_b = (((r < M) & (c >= L))
              | ((r >= M) & (r < 32) & (c >= L) & (c <= r + 48))
              | ((r >= 32) & (r < L) & (c <= r))
              | ((r >= L) & (mem_b | ((c >= L) & (c <= r)))))
    exp_c = (DH ** -0.5) * math.log2(math.e)
    neg = -1e9 * DH ** 0.5

    def proj(lhs, m, h, k0=0, k1=D):
        idx = m * H + (h % 2) * 16 + h // 2
        r0 = W0 + idx * SLAB - 4 * (idx % 2)
        w = pltpu.bitcast(w_s[r0 + k0 // 2:r0 + k1 // 2, :], BF16)
        return jnp.dot(lhs[idx % 2][:, k0:k1], w, preferred_element_type=F32)

    HEADS = [h for h in range(H) if (h // 2) % 2 == 0] + [h for h in range(H) if (h // 2) % 2 == 1]
    G = 4
    H_SPLIT = 2
    H_EARLY = 20

    def segment(lhs, first):
        qs, ks, vs, ps = {}, {}, {}, {}
        prow = lhs.shape[0]
        lhs = (lhs, pltpu.bitcast(pltpu.roll(pltpu.bitcast(lhs, U32), 8, 1), BF16))

        def stage_p(h):
            if h < H_SPLIT:
                q, k, v = (jnp.concatenate([r[0:8] + pre_s[i, 0:8, :], r[8:] + pre_s[i, 8:prow, :]],
                                           axis=0).astype(BF16)
                           for i, r in ((3 * h + m, proj(lhs, m, h, D // 2, D)) for m in range(3)))
            else:
                q, k, v = (proj(lhs, m, h).astype(BF16) for m in range(3))
            if first:
                sv_s[h, 0:8, :] = pltpu.bitcast(q[32:48], U32)
                sv_s[h, 8:32, :] = pltpu.bitcast(k, U32)
                sv_s[h, 32:56, :] = pltpu.bitcast(v, U32)
                q = q[0:32]
            else:
                q = jnp.concatenate([q, pltpu.bitcast(sv_s[h, 0:8, :], BF16)], axis=0)
                k = jnp.concatenate([pltpu.bitcast(sv_s[h, 8:32, :], BF16), k], axis=0)
                v = jnp.concatenate([pltpu.bitcast(sv_s[h, 32:56, :], BF16), v], axis=0)
            qs[h], ks[h], vs[h] = q, k, v

        def stage_s(h):
            s = jax.lax.dot_general(qs.pop(h), ks.pop(h), NT, preferred_element_type=F32)
            s = jnp.where(mask_a if first else mask_b, s, neg)
            mx = jnp.max(s, axis=-1, keepdims=True)
            p = jnp.exp2((s - mx) * exp_c)
            l = jnp.sum(p, axis=-1, keepdims=True)
            r = pl.reciprocal(l, approx=True)
            r = r * (2.0 - l * r)
            ps[h] = (p * r).astype(BF16)

        rows = 32 if first else 48

        def stage_v(h):
            o = jnp.dot(ps.pop(h), vs.pop(h), preferred_element_type=F32)
            o_s[h, 0:rows // 2, :] = pltpu.bitcast(o.astype(BF16), U32)

        def wo_part(n, h0, h1):
            o = jnp.concatenate([pltpu.bitcast(o_s[h, 0:rows // 2, :], BF16) for h in HEADS[h0:h1]], axis=1)
            w = jnp.concatenate([wo_s[n * WOP + h * DH // 2:n * WOP + (h + 1) * DH // 2, :]
                                 for h in HEADS[h0:h1]], axis=0)
            return jnp.dot(o, pltpu.bitcast(w, BF16), preferred_element_type=F32)

        def wo_early(n):
            acc_s[0:rows, n * 128:(n + 1) * 128] = wo_part(n, 0, H_EARLY)

        def group(stage, last):
            for i in range(max(last - G + 1, 0), min(last + 1, H)):
                stage(HEADS[i])

        for h in range(H_SPLIT):
            for m in range(3):
                pre_s[3 * h + m, 0:prow, :] = proj(lhs, m, h, 0, D // 2)
        for i in range(H):
            stage_p(HEADS[i])
            if i % G == G - 1:
                group(stage_v, i - 1 - G)
                group(stage_s, i - 1)
        wo_early(0)
        group(stage_s, H - 2 + G)
        wo_early(1)
        wo_early(2)
        group(stage_v, H - 2)
        wo_early(3)
        wo_early(4)
        group(stage_v, H - 2 + G)
        for n in range(5, NB):
            wo_early(n)
        late = jnp.concatenate([wo_part(n, H_EARLY, H) for n in range(NB)], axis=1)
        return jnp.concatenate([late[0:M] + acc_s[0:M, :], late[M:rows] + acc_s[M:rows, :]], axis=0)

    def b_pair(j, mem):
        base = pl.multiple_of(j * PAIR, PAIR)
        x = xb_s[pl.ds(base, PAIR), :].astype(F32)
        lhs = jnp.concatenate([mem, x[0:40]], axis=0).astype(BF16)
        res = segment(lhs, True)
        ob_s[pl.ds(base, 24), :] = res[8:32]
        lhs = jnp.concatenate([res[0:M], x[40:64]], axis=0).astype(BF16)
        res = segment(lhs, False)
        ob_s[pl.ds(base + 40, 24), :] = res[8:32]
        ob_s[pl.ds(base + 24, 16), :] = res[32:48]
        pltpu.make_async_copy(ob_s.at[pl.ds(base, PAIR), :],
                              out_hbm.at[pl.ds(base, PAIR), pl.ds(D, D)],
                              out_sem.at[1]).start()
        return res[0:M]

    def b_body(j, mem):
        for u in range(B_UNROLL):
            mem = b_pair(j * B_UNROLL + u, mem)
        return mem

    jax.lax.fori_loop(0, N_PAIR // B_UNROLL, b_body, mem0_s[...].astype(F32))

    pltpu.make_async_copy(ya_s, out_hbm.at[:, pl.ds(0, D)], out_sem.at[0]).wait()
    pltpu.make_async_copy(ob_s, out_hbm.at[:, pl.ds(D, D)], out_sem.at[1]).wait()


@jax.jit
def _run(A_x, A_Lambda_re, A_Lambda_im, A_B_re, A_B_im, A_C_re, A_C_im, A_log_dt, A_Dskip,
         B_x, B_mem0, B_Wq, B_Wk, B_Wv, B_Wo):
    hbm = pl.BlockSpec(memory_space=pl.ANY)
    out = pl.pallas_call(
        _kernel,
        out_shape=jax.ShapeDtypeStruct((S, 2 * D), F32),
        in_specs=[hbm] * 15,
        out_specs=hbm,
        scratch_shapes=[
            pltpu.VMEM((S, D), BF16),
            pltpu.VMEM((S, D), BF16),
            pltpu.VMEM((4 * D, D), BF16),
            pltpu.VMEM((3, D * H, DH), BF16),
            pltpu.VMEM((H * DH, D), BF16),
            pltpu.VMEM((W0 + 3 * H * SLAB + 520, 128), U32),
            pltpu.VMEM((NB * WOP + 8, 128), U32),
            pltpu.VMEM(((2 * NB + 1) * HP, 128), U32),
            pltpu.VMEM((S, D), F32),
            pltpu.VMEM((S, D), F32),
            pltpu.VMEM(((2 * NB + 1) * TAP, 128), F32),
            pltpu.VMEM(((2 * NB + 1) * TAP, 128), F32),
            pltpu.VMEM((H, 56, 128), U32),
            pltpu.VMEM((H, 24, 128), U32),
            pltpu.VMEM((48, D), F32),
            pltpu.VMEM((6, 48, 128), F32),
            pltpu.VMEM((4, NB, 128), BF16),
            pltpu.VMEM((M, D), BF16),
            pltpu.SMEM((1,), jnp.int32),
            pltpu.SemaphoreType.DMA((32 + 4 * NQ,)),
            pltpu.SemaphoreType.DMA((2,)),
        ],
        compiler_params=pltpu.CompilerParams(vmem_limit_bytes=120 * 1024 * 1024, disable_bounds_checks=True, disable_semaphore_checks=True),
    )(
        A_x.reshape(S, D),
        A_Lambda_re.reshape(NB, 128),
        A_Lambda_im.reshape(NB, 128),
        A_B_re, A_B_im, A_C_re, A_C_im,
        A_log_dt.reshape(NB, 128),
        A_Dskip.reshape(NB, 128),
        B_x.reshape(S, D),
        B_mem0.reshape(M, D),
        B_Wq.reshape(D * H, DH),
        B_Wk.reshape(D * H, DH),
        B_Wv.reshape(D * H, DH),
        B_Wo.reshape(H * DH, D),
    )
    return out.reshape(1, S, 2 * D)


def pallas_concat_heads__ssm_conv_s5__memory_aug_recurrent_mem_tr__prompt_kernel(
    A_x: jax.Array,
    A_Lambda_re: jax.Array,
    A_Lambda_im: jax.Array,
    A_B_re: jax.Array,
    A_B_im: jax.Array,
    A_C_re: jax.Array,
    A_C_im: jax.Array,
    A_log_dt: jax.Array,
    A_Dskip: jax.Array,
    B_x: jax.Array,
    B_mem0: jax.Array,
    B_Wq: jax.Array,
    B_Wk: jax.Array,
    B_Wv: jax.Array,
    B_Wo: jax.Array,
    B_seg_len,
):
    if isinstance(B_seg_len, int):
        assert B_seg_len == SEG
    assert A_x.shape == (1, S, D) and B_x.shape == (1, S, D)
    assert B_Wq.shape == (D, H, DH) and B_Wo.shape == (H, DH, D) and B_mem0.shape == (1, M, D)
    return _run(A_x, A_Lambda_re, A_Lambda_im, A_B_re, A_B_im, A_C_re, A_C_im, A_log_dt, A_Dskip,
                B_x, B_mem0, B_Wq, B_Wk, B_Wv, B_Wo)
```

```python
import math

import jax
import jax.numpy as jnp
import jax.experimental.pallas as pl
import jax.experimental.pallas.tpu as pltpu

F32 = jnp.float32
BF16 = jnp.bfloat16
U32 = jnp.uint32

S = 2048
D = 1024
H = 32
DH = 128
M = 8
SEG = 32
L = M + SEG
NB = D // 128
PAIR = 2 * SEG
N_PAIR = S // PAIR
B_UNROLL = 2

SLAB = 516
W0 = 8
TA = 128
TAP = TA + 8
N_CH = S // TA
NQ = 8
TY = S // NQ
HP = S // 2 + 8
WOP = H * DH // 2

B_GROUPS = ((0, 2), (2, 4), (4, 6), (6, 8), (8, 10), (10, 13), (13, 16))

NT = (((1,), (1,)), ((), ()))


def _kernel(xa_hbm, lre_hbm, lim_hbm, bre_hbm, bim_hbm, cre_hbm, cim_hbm, ldt_hbm, dsk_hbm,
            xb_hbm, mem0_hbm, wq_hbm, wk_hbm, wv_hbm, wo_hbm,
            out_hbm,
            xa_s, xb_s, bc_s, wraw_s, woraw_s, w_s, wo_s, h_s, ya_s, ob_s,
            sb0, sb1, sv_s, o_s, o8_s, acc_s, pre_s, par_s, mem0_s, z_s,
            in_sem, out_sem):
    def cp_xa(i):
        r0 = pl.multiple_of(i * (2 * TA), 2 * TA)
        return pltpu.make_async_copy(xa_hbm.at[pl.ds(r0, 2 * TA), :], xa_s.at[pl.ds(r0, 2 * TA), :],
                                     in_sem.at[10 + i])

    def cp_b(g, src=None):
        if isinstance(g, int):
            rows = pl.ds(B_GROUPS[g][0] * 128, (B_GROUPS[g][1] - B_GROUPS[g][0]) * 128)
        else:
            rows = pl.ds(pl.multiple_of(g * 256, 256), 256)
        dst = bc_s.at[rows, :]
        return pltpu.make_async_copy(dst if src is None else src, dst, in_sem.at[18 + g])

    cp_small = [pltpu.make_async_copy(src, dst, in_sem.at[2 + i]) for i, (src, dst) in enumerate(
        ((lre_hbm, par_s.at[0]), (lim_hbm, par_s.at[1]), (ldt_hbm, par_s.at[2]), (dsk_hbm, par_s.at[3]),
         (mem0_hbm, mem0_s)))]
    cp_c = [pltpu.make_async_copy(src, bc_s.at[pl.ds((2 + i) * D, D), :], in_sem.at[7 + i])
            for i, src in enumerate((cre_hbm, cim_hbm))]
    cp_xb = pltpu.make_async_copy(xb_hbm, xb_s, in_sem.at[9])
    wrows = D * H // NQ
    worows = H * DH // NQ

    def cp_w(m, c):
        if m == 3:
            return pltpu.make_async_copy(wo_hbm.at[pl.ds(c * worows, worows), :],
                                         woraw_s.at[pl.ds(c * worows, worows), :],
                                         in_sem.at[32 + c * 4 + m])
        src = (wq_hbm, wk_hbm, wv_hbm)[m]
        return pltpu.make_async_copy(src.at[pl.ds(c * wrows, wrows), :],
                                     wraw_s.at[m, pl.ds(c * wrows, wrows), :],
                                     in_sem.at[32 + c * 4 + m])

    cp_xa(0).start()
    for g, (b0, b1) in enumerate(B_GROUPS):
        cp_b(g, (bre_hbm, bim_hbm)[b0 // NB].at[pl.ds(b0 % NB * 128, (b1 - b0) * 128), :]).start()
        if g == 4:
            for c in cp_small:
                c.start()
    for i in range(1, N_CH // 2):
        cp_xa(i).start()
    for c in cp_c:
        c.start()
    for c in range(NQ):
        for m in range(4):
            cp_w(m, c).start()
    cp_xb.start()

    scan_bufs = (sb0, sb1)
    z_s[0] = 0
    zrow = {id(w_s): W0 + 3 * H * SLAB, id(wo_s): NB * WOP, id(h_s): 2 * NB * HP}
    for ref in (w_s, wo_s, h_s):
        ref[zrow[id(ref)]:zrow[id(ref)] + 8, :] = jnp.zeros((8, 128), ref.dtype)

    def token(*refs):
        tok = None
        for ref in refs:
            t = ref[pl.ds(pl.multiple_of(zoff + zrow[id(ref)], 8), 8), :]
            tok = t if tok is None else tok | t
        return tok

    def after(blocks, toks):
        blocks = list(blocks)
        for b, tok in toks.items():
            blocks[b] = jnp.concatenate([blocks[b][0:8] | tok, blocks[b][8:]], axis=0)
        return jnp.concatenate([pltpu.bitcast(b, BF16) for b in blocks], axis=1)

    def pack2(a, b):
        r = pltpu.bitcast(jnp.concatenate([a, b], axis=0).astype(BF16).astype(F32), U32)
        return (r[0:8] >> 16) | (r[8:16] & jnp.uint32(0xFFFF0000))

    def scan_steps(c, u, t0, t1, gr, gi, toff=0):
        sb = scan_bufs[u]
        for t in range(t0, t1, 2):
            out = []
            for tt in (t, t + 1):
                ur = sb[pl.ds(toff + tt, NB, stride=TAP), :]
                ui = sb[pl.ds(toff + tt + NB * TAP, NB, stride=TAP), :]
                vr = cf_re * ur - cf_im * ui
                vi = cf_re * ui + cf_im * ur
                gr, gi = (lb_re * gr + lb_im * gi) + vr, (lb_re * gi - lb_im * gr) - vi
                out.append((gr, gi))
            row = c * (TA // 2) + (toff + t) // 2
            h_s[pl.ds(row, NB, stride=HP), :] = pack2(out[0][0], out[1][0])
            h_s[pl.ds(row + NB * HP, NB, stride=HP), :] = pack2(out[0][1], out[1][1])
        return gr, gi

    SCAN_END = [min(TA, 2 * -(-(k + 1) * TA // 2 // 13)) for k in range(2 * NB)]

    def bu_and_scan(cb, ub, cs, us, gr, gi):
        r0 = pl.multiple_of(cb * TA, TA)
        xblk = [pltpu.bitcast(xa_s[pl.ds(r0, TA), n * 128:(n + 1) * 128], U32) for n in range(NB)]
        zero_bits = token(h_s)
        toks = [{}, {}]
        done = 0
        for i in range(2 * NB):
            r = jax.lax.dot_general(after(xblk, toks.pop(0)), bc_s[i * 128:(i + 1) * 128, :], NT,
                                    preferred_element_type=F32)
            scan_bufs[ub][i * TAP:i * TAP + TA, :] = r
            toks.append({})
            if done < SCAN_END[i]:
                gr = gr + pltpu.bitcast(pltpu.bitcast(r[0:8], U32) & zero_bits, F32)
                gr, gi = scan_steps(cs, us, done, SCAN_END[i], gr, gi)
                done = SCAN_END[i]
                toks[1] = {4: token(h_s)}
        assert done == TA
        return gr, gi

    def bu_dot(c, b):
        w0, s0 = b * 128, b * TAP
        if not isinstance(b, int):
            w0, s0 = pl.multiple_of(w0, 128), pl.multiple_of(s0, 8)
        r = jax.lax.dot_general(xa_s[c * TA:(c + 1) * TA, :], bc_s[pl.ds(w0, 128), :], NT,
                                preferred_element_type=F32)
        scan_bufs[c][pl.ds(s0, TA), :] = r
        return r

    def pro_body(g, carry):
        cp_b(g).wait()
        for b in (2 * g, 2 * g + 1):
            for c in range(2):
                bu_dot(c, b)
        return carry

    cp_xa(0).wait()
    jax.lax.fori_loop(0, 5, pro_body, 0)
    cp_b(5).wait()
    for c in cp_small:
        c.wait()
    zoff = z_s[0]
    lre = par_s[0].astype(F32)
    lim = par_s[1].astype(F32)
    dt = jnp.exp(par_s[2].astype(F32)).astype(BF16).astype(F32)
    mag = jnp.exp(dt * lre)
    ang = dt * lim
    lb_re = mag * jnp.cos(ang)
    lb_im = mag * jnp.sin(ang)
    nr = lb_re - 1.0
    den = lre * lre + lim * lim
    cf_re = 2.0 * (nr * lre + lb_im * lim) / den
    cf_im = 2.0 * (lb_im * lre - nr * lim) / den
    dsk = par_s[3].astype(F32)
    for c, b in ((0, 10), (0, 11), (0, 12), (1, 10), (1, 11)):
        bu_dot(c, b)
    cp_b(6).wait()
    for b in (13, 14, 15):
        bu_dot(0, b)
    gr = gi = jnp.zeros((NB, 128), F32)
    zero_bits = token(h_s)
    for b, t0, t1 in ((12, 0, 16), (13, 16, 52), (14, 52, 90), (15, 90, TA)):
        r = bu_dot(1, b)
        gr, gi = scan_steps(0, 0, t0, t1, gr, gi)
        gr = gr + pltpu.bitcast(pltpu.bitcast(r[0:8], U32) & zero_bits, F32)
    g0 = (gr, gi)

    def a1_body(i, carry):
        cp_xa(i).wait()
        gr, gi = carry
        gr, gi = bu_and_scan(2 * i, 0, 2 * i - 1, 1, gr, gi)
        gr, gi = bu_and_scan(2 * i + 1, 1, 2 * i, 0, gr, gi)
        return gr, gi

    g1 = jax.lax.fori_loop(1, N_CH // 2, a1_body, g0)
    for c in cp_c:
        c.wait()

    def a2_body(q, carry):
        for m in range(4):
            cp_w(m, q).wait()
        npair = D // 2 // NQ
        gr, gi = carry

        def rl_w(u):
            dp = q * npair + u
            rows = [dp]
            if u >= npair - 4:
                rows.append(jnp.where(q == NQ - 1, dp - D // 2, dp))
            for m in range(3):
                w = pltpu.bitcast(wraw_s[m, pl.ds(pl.multiple_of(dp * 64, 64), 64), :], U32)
                e = w[0:16]
                o = w[16:32]
                lo = (e & jnp.uint32(0xFFFF)) | (o << 16)
                hi = (e >> 16) | (o & jnp.uint32(0xFFFF0000))
                for r in rows:
                    w_s[pl.ds(W0 + m * H * SLAB + r, 16, stride=SLAB), :] = lo
                    w_s[pl.ds(W0 + (m * H + 16) * SLAB + r, 16, stride=SLAB), :] = hi

        def rl_wo(u):
            r0 = pl.multiple_of(q * worows + (u // 4) * 32, 32)
            r1 = pl.multiple_of(q * (worows // 2) + (u // 4) * 16, 16)
            for n in range(2 * (u % 4), 2 * (u % 4) + 2):
                wo_s[pl.ds(n * WOP + r1, 16), :] = pltpu.bitcast(
                    woraw_s[pl.ds(r0, 32), n * 128:(n + 1) * 128], U32)

        todo = list(range(npair))

        def piece():
            for _ in range(2 if len(todo) % (npair // 4) == 0 else 1):
                u = todo.pop(0)
                rl_w(u)
                rl_wo(u)
            return token(w_s, wo_s)

        toks_r, toks_i = {}, {}
        zero_bits = jnp.concatenate([token(h_s)] * (TA // 16), axis=0)
        for u in range(TY // TA):
            base = pl.multiple_of(q * TY + u * TA, TA)
            hb = pl.multiple_of(q * (TY // 2) + u * (TA // 2), TA // 2)
            hr = [h_s[pl.ds(n * HP + hb, TA // 2), :] for n in range(NB)]
            hi = [h_s[pl.ds((NB + n) * HP + hb, TA // 2), :] for n in range(NB)]
            hr = [v | zero_bits for v in hr]
            hi = [v | zero_bits for v in hi]
            for n in range(NB):
                y = jax.lax.dot_general(after(hr, toks_r), bc_s[2 * D + n * 128:2 * D + (n + 1) * 128, :], NT,
                                        preferred_element_type=F32)
                y = y + jax.lax.dot_general(after(hi, toks_i), bc_s[3 * D + n * 128:3 * D + (n + 1) * 128, :], NT,
                                            preferred_element_type=F32)
                y = y + xa_s[pl.ds(base, TA), n * 128:(n + 1) * 128].astype(F32) * dsk[n:n + 1, :]
                ya_s[pl.ds(base, TA), n * 128:(n + 1) * 128] = y
                if u == 0 and n < TA // NQ // 4:
                    gr = gr + pltpu.bitcast(pltpu.bitcast(y[0:8], U32) & zero_bits[0:8], F32)
                    gr, gi = scan_steps(N_CH - 1, 1, 4 * n, 4 * n + 4, gr, gi, q * (TA // NQ))
                if todo:
                    toks_i = {0: piece(), 4: piece()}
                    toks_r = {0: piece(), 4: piece()}
        assert not todo
        base = pl.multiple_of(q * TY, TY)
        pltpu.make_async_copy(ya_s.at[pl.ds(base, TY), :],
                              out_hbm.at[pl.ds(base, TY), pl.ds(0, D)],
                              out_sem.at[0]).start()
        return gr, gi

    jax.lax.fori_loop(0, NQ, a2_body, g1)
    cp_xb.wait()

    r = jax.lax.broadcasted_iota(jnp.int32, (32, 48), 0)
    c = jax.lax.broadcasted_iota(jnp.int32, (32, 48), 1)
    own = (c < 32) & ((r < M) | (r >= c))
    mask_a = own | ((c >= 32) & (c < L))
    mask_b = own | (c >= L)
    row8 = jax.lax.broadcasted_iota(jnp.int32, (8, 1), 0)
    exp_c = (DH ** -0.5) * math.log2(math.e)
    neg = -1e9 * DH ** 0.5

    def recip(l):
        r = pl.reciprocal(l, approx=True)
        return r * (2.0 - l * r)

    def gate(a, toks):
        if not toks:
            return a
        u = pltpu.bitcast(a, U32)
        return after([u[:, b * 128:(b + 1) * 128] for b in range(a.shape[1] // 128)], toks)

    def proj(lhs, m, h, k0=0, k1=D, toks=None):
        idx = m * H + (h % 2) * 16 + h // 2
        r0 = W0 + idx * SLAB - 4 * (idx % 2)
        w = pltpu.bitcast(w_s[r0 + k0 // 2:r0 + k1 // 2, :], BF16)
        return jnp.dot(gate(lhs[idx % 2][:, k0:k1], toks), w, preferred_element_type=F32)

    def attend8(q, km, kx, vm, vx):
        q = q * exp_c
        sc = [jnp.sum(q * km[j:j + 1], axis=-1, keepdims=True) for j in range(8)]
        for j in range(8):
            t = jnp.sum(q * kx[j:j + 1], axis=-1, keepdims=True)
            sc.append(t if j == 0 else jnp.where(row8 >= j, t, neg * exp_c))
        mx = sc[0]
        for t in sc[1:]:
            mx = jnp.maximum(mx, t)
        p = [jnp.exp2(t - mx) for t in sc]
        l = p[0]
        o = p[0] * vm[0:1]
        for j in range(1, 16):
            l = l + p[j]
            o = o + p[j] * (vm[j:j + 1] if j < 8 else vx[j - 8:j - 7])
        return o * recip(l)

    HEADS = [h for h in range(H) if (h // 2) % 2 == 0] + [h for h in range(H) if (h // 2) % 2 == 1]
    G = 4
    H_SPLIT = 2
    H_EARLY = 24
    H_MIX = 16
    MIX0 = 9
    T_LAG = 4
    H_P = H - T_LAG
    S_POS, V_POS = 1, 5

    def segment(lhs, first, zero_bits):
        qs, ks, vs, ps, toks = {}, {}, {}, {}, {}
        prow = lhs.shape[0]
        h_mix = 0 if first else H_MIX
        p_due = {}
        for i in range(H_P):
            t = T_LAG + i
            if not first and i >= G:
                t = max(t, MIX0 + (i - G) * (H - MIX0) // (H_P - G))
            p_due.setdefault(t, []).append(i)
        kslots = (H_EARLY - h_mix) // 4
        w_due = {divmod(((i - H_P + 1) * NB * kslots - 1) // (H - H_P), kslots): i for i in range(H_P, H)}
        lhs = (lhs, pltpu.bitcast(pltpu.roll(pltpu.bitcast(lhs, U32), 8, 1), BF16))

        def stage_p(i):
            h = HEADS[i]
            if h < H_SPLIT:
                q, k, v = (jnp.concatenate([r[0:8] + pre_s[j, 0:8, :], r[8:] + pre_s[j, 8:prow, :]],
                                           axis=0).astype(BF16)
                           for j, r in ((3 * h + m, proj(lhs, m, h, D // 2, D)) for m in range(3)))
            else:
                due = {2 - j: {0: toks.pop(t)} for j, t in enumerate(reversed(p_due.get(i, [])))}
                q, k, v = (proj(lhs, m, h, toks=due.get(m)).astype(BF16) for m in range(3))
            km, vm = k[0:16].astype(F32)[0:8], v[0:16].astype(F32)[0:8]
            if first:
                q16, k16, v16 = q[32:48], k[32:48], v[32:48]
                for j, a in enumerate((q16, k16, v16)):
                    sv_s[h, 8 * j:8 * j + 8, :] = pltpu.bitcast(a, U32)
                q = q[0:32]
                lo = 0
            else:
                q16, k16, v16 = (pltpu.bitcast(sv_s[h, 8 * j:8 * j + 8, :], BF16) for j in range(3))
                k = jnp.concatenate([k, k16], axis=0)
                v = jnp.concatenate([v, v16], axis=0)
                lo = 8
            qx, kx, vx = (a.astype(F32)[lo:lo + 8] for a in (q16, k16, v16))
            o8 = attend8(qx, km, kx, vm, vx)
            if first:
                o8_s[h] = o8
                bits = pltpu.bitcast(o8, U32)
            else:
                bits = pltpu.bitcast(jnp.concatenate([o8_s[h], o8], axis=0).astype(BF16), U32)
                o_s[h, 16:24, :] = bits
            toks[i] = bits & zero_bits
            qs[h], ks[h], vs[h] = q, k, v

        def stage_s(h):
            s = jax.lax.dot_general(qs.pop(h), ks.pop(h), NT, preferred_element_type=F32)
            s = jnp.where(mask_a if first else mask_b, s, neg)
            mx = jnp.max(s, axis=-1, keepdims=True)
            p = jnp.exp2((s - mx) * exp_c)
            ps[h] = (p * recip(jnp.sum(p, axis=-1, keepdims=True))).astype(BF16)

        rows = 32 if first else 48
        done = set()

        def stage_v(h):
            done.add(h)
            o = jnp.dot(ps.pop(h), vs.pop(h), preferred_element_type=F32)
            o_s[h, 0:16, :] = pltpu.bitcast(o.astype(BF16), U32)

        def wo_part(n, h0, h1, toks=None):
            assert done.issuperset(HEADS[h0:h1])
            o = jnp.concatenate([pltpu.bitcast(o_s[h, 0:rows // 2, :], BF16) for h in HEADS[h0:h1]], axis=1)
            w = jnp.concatenate([wo_s[n * WOP + h * DH // 2:n * WOP + (h + 1) * DH // 2, :]
                                 for h in HEADS[h0:h1]], axis=0)
            return jnp.dot(gate(o, toks), pltpu.bitcast(w, BF16), preferred_element_type=F32)

        def acc_add(r, cols):
            return jnp.concatenate([r[0:M] + acc_s[0:M, cols], r[M:rows] + acc_s[M:rows, cols]], axis=0)

        def wo_acc(n, h0, h1, due=None):
            cols = slice(n * 128, (n + 1) * 128)
            r = wo_part(n, h0, h1, due)
            acc_s[0:rows, cols] = r if h0 == 0 else acc_add(r, cols)

        def wo_early(n):
            due = {4 * kg: toks.pop(i) for (nn, kg), i in w_due.items() if nn == n}
            wo_acc(n, h_mix, H_EARLY, due)

        def group(stage, g):
            if 0 <= g < H // G:
                for i in range(g * G, g * G + G):
                    stage(HEADS[i])

        for h in range(H_SPLIT):
            for m in range(3):
                pre_s[3 * h + m, 0:prow, :] = proj(lhs, m, h, 0, D // 2)
        mix = [(n, g * G, g * G + G) for g in range(h_mix // G) for n in range(NB)]
        nmix = len(mix)
        for i in range(H):
            stage_p(i)
            if i % G == 0:
                group(stage_v, i // G - 2)
                group(stage_s, i // G - 1)
            while i >= MIX0 and nmix - len(mix) < nmix * (i - MIX0 + 1) // (H - MIX0):
                wo_acc(*mix.pop(0))
        group(stage_v, H // G - 2)
        for n in range(NB):
            wo_early(n)
            if n == S_POS:
                group(stage_s, H // G - 1)
            if n == V_POS:
                group(stage_v, H // G - 1)
        assert not toks and not mix
        late = jnp.concatenate([wo_part(n, H_EARLY, H) for n in range(NB)], axis=1)
        return acc_add(late, slice(None))

    def b_pair(j, mem):
        base = pl.multiple_of(j * PAIR, PAIR)
        zero_bits = token(h_s)
        x = xb_s[pl.ds(base, PAIR), :].astype(F32)
        lhs = jnp.concatenate([mem, x[8:32], x[0:8], x[32:40]], axis=0).astype(BF16)
        res = segment(lhs, True, zero_bits)
        ob_s[pl.ds(base + 8, 24), :] = res[8:32]
        lhs = jnp.concatenate([res[0:M], x[40:64]], axis=0).astype(BF16)
        res = segment(lhs, False, zero_bits)
        ob_s[pl.ds(base + 40, 24), :] = res[8:32]
        ob_s[pl.ds(base, 8), :] = res[32:40]
        ob_s[pl.ds(base + 32, 8), :] = res[40:48]
        pltpu.make_async_copy(ob_s.at[pl.ds(base, PAIR), :],
                              out_hbm.at[pl.ds(base, PAIR), pl.ds(D, D)],
                              out_sem.at[1]).start()
        return res[0:M]

    def b_body(j, mem):
        for u in range(B_UNROLL):
            mem = b_pair(j * B_UNROLL + u, mem)
        return mem

    jax.lax.fori_loop(0, N_PAIR // B_UNROLL, b_body, mem0_s[...].astype(F32))
    pltpu.make_async_copy(ya_s, out_hbm.at[:, pl.ds(0, D)], out_sem.at[0]).wait()
    pltpu.make_async_copy(ob_s, out_hbm.at[:, pl.ds(D, D)], out_sem.at[1]).wait()


@jax.jit
def _run(A_x, A_Lambda_re, A_Lambda_im, A_B_re, A_B_im, A_C_re, A_C_im, A_log_dt, A_Dskip,
         B_x, B_mem0, B_Wq, B_Wk, B_Wv, B_Wo):
    hbm = pl.BlockSpec(memory_space=pl.ANY)
    out = pl.pallas_call(
        _kernel,
        out_shape=jax.ShapeDtypeStruct((S, 2 * D), F32),
        in_specs=[hbm] * 15,
        out_specs=hbm,
        scratch_shapes=[
            pltpu.VMEM((S, D), BF16),
            pltpu.VMEM((S, D), BF16),
            pltpu.VMEM((4 * D, D), BF16),
            pltpu.VMEM((3, D * H, DH), BF16),
            pltpu.VMEM((H * DH, D), BF16),
            pltpu.VMEM((W0 + 3 * H * SLAB + 520, 128), U32),
            pltpu.VMEM((NB * WOP + 8, 128), U32),
            pltpu.VMEM(((2 * NB + 1) * HP, 128), U32),
            pltpu.VMEM((S, D), F32),
            pltpu.VMEM((S, D), F32),
            pltpu.VMEM(((2 * NB + 1) * TAP, 128), F32),
            pltpu.VMEM(((2 * NB + 1) * TAP, 128), F32),
            pltpu.VMEM((H, 24, 128), U32),
            pltpu.VMEM((H, 24, 128), U32),
            pltpu.VMEM((H, 8, 128), F32),
            pltpu.VMEM((48, D), F32),
            pltpu.VMEM((6, 48, 128), F32),
            pltpu.VMEM((4, NB, 128), BF16),
            pltpu.VMEM((M, D), BF16),
            pltpu.SMEM((1,), jnp.int32),
            pltpu.SemaphoreType.DMA((32 + 4 * NQ,)),
            pltpu.SemaphoreType.DMA((2,)),
        ],
        compiler_params=pltpu.CompilerParams(vmem_limit_bytes=120 * 1024 * 1024,
                                             disable_bounds_checks=True,
                                             disable_semaphore_checks=True),
    )(
        A_x.reshape(S, D),
        A_Lambda_re.reshape(NB, 128),
        A_Lambda_im.reshape(NB, 128),
        A_B_re, A_B_im, A_C_re, A_C_im,
        A_log_dt.reshape(NB, 128),
        A_Dskip.reshape(NB, 128),
        B_x.reshape(S, D),
        B_mem0.reshape(M, D),
        B_Wq.reshape(D * H, DH),
        B_Wk.reshape(D * H, DH),
        B_Wv.reshape(D * H, DH),
        B_Wo.reshape(H * DH, D),
    )
    return out.reshape(1, S, 2 * D)


def pallas_concat_heads__ssm_conv_s5__memory_aug_recurrent_mem_tr__prompt_kernel(
    A_x: jax.Array,
    A_Lambda_re: jax.Array,
    A_Lambda_im: jax.Array,
    A_B_re: jax.Array,
    A_B_im: jax.Array,
    A_C_re: jax.Array,
    A_C_im: jax.Array,
    A_log_dt: jax.Array,
    A_Dskip: jax.Array,
    B_x: jax.Array,
    B_mem0: jax.Array,
    B_Wq: jax.Array,
    B_Wk: jax.Array,
    B_Wv: jax.Array,
    B_Wo: jax.Array,
    B_seg_len,
):
    if isinstance(B_seg_len, int):
        assert B_seg_len == SEG
    assert A_x.shape == (1, S, D) and B_x.shape == (1, S, D)
    assert B_Wq.shape == (D, H, DH) and B_Wo.shape == (H, DH, D) and B_mem0.shape == (1, M, D)
    return _run(A_x, A_Lambda_re, A_Lambda_im, A_B_re, A_B_im, A_C_re, A_C_im, A_log_dt, A_Dskip,
                B_x, B_mem0, B_Wq, B_Wk, B_Wv, B_Wo)
```
